```python
import jax
import jax.numpy as jnp

def _softmax(x, axis=-1):
    return jax.nn.softmax(x, axis=axis)
def _gelu(x):
    return jax.nn.gelu(x, approximate=True)
def _silu(x):
    return jax.nn.silu(x)
def _sigmoid(x):
    return jax.nn.sigmoid(x)
def _layernorm(x, axis=-1, eps=1e-5):
    m = jnp.mean(x, axis=axis, keepdims=True)
    v = jnp.var(x, axis=axis, keepdims=True)
    return (x - m) / jnp.sqrt(v + eps)
def _scatter_add(tgt, idx, src, axis=0):
    return tgt.at[idx].add(src)
def _segment_sum(src, seg, n):
    return jax.ops.segment_sum(src, seg, n)
class _Rng:
    def __init__(self, key):
        self._k = key
    def _next(self):
        self._k, sub = jax.random.split(self._k)
        return sub
    def normal(self, shape):
        return jax.random.normal(self._next(), shape, dtype=jnp.bfloat16)
    def randint(self, lo, hi, shape):
        return jax.random.randint(self._next(), shape, lo, hi, dtype=jnp.int32)
    def uniform(self, shape, lo=0.0, hi=1.0):
        return jax.random.uniform(self._next(), shape, jnp.bfloat16, lo, hi)
    def permutation(self, n):
        return jax.random.permutation(self._next(), n)


kernel_name = 'standalone__instancenorm__prompt'

def setup_inputs():
    _rng = _Rng(jax.random.key(int.from_bytes(__import__("os").urandom(4), "little")))
    _w = (lambda a: (lambda t: t.astype(jnp.bfloat16) if jnp.issubdtype(t.dtype, jnp.floating) else t)(jnp.asarray(a)))
    B, C, H, W = 2, 1024, 2048, 32
    return {
        "x": _w((lambda *s: _rng.normal(s) * 0.05)(B, C, H, W)),
        "g": _w((lambda *s: _rng.normal(s) * 0.05)(C) + 1.0),
        "b": _w((lambda *s: _rng.normal(s) * 0.05)(C)),
    }

def reference(x, g, b):
    mu = x.mean(axis=(-2, -1), keepdims=True)
    var = ((x - mu) * (x - mu)).mean(axis=(-2, -1), keepdims=True)
    xhat = (x - mu) / jnp.sqrt(var + 1e-5)
    return xhat * g.reshape(1, -1, 1, 1) + b.reshape(1, -1, 1, 1)
```

```python
import jax
import jax.numpy as jnp
from jax import lax
from jax.experimental import pallas as pl
from jax.experimental.pallas import tpu as pltpu

_EPS = 1e-5
_LANES = 128


@jax.jit
def pallas_standalone__instancenorm__prompt_kernel(
    x: jax.Array,
    g: jax.Array,
    b: jax.Array,
):
    B, C, H, W = x.shape
    N = B * C
    S = 64
    J = 8
    RP = 8
    U = 2
    CH = 512
    M = 5
    A = N // (S * J)
    R = W // RP
    assert A * S * J == N and R * RP == W and H % CH == 0 and C % _LANES == 0
    inv_n = 1.0 / (H * W)
    nch = H // CH

    xt = jnp.transpose(x, (0, 1, 3, 2)).reshape(A, S, J, R, RP, H)
    g2 = g.reshape(C // _LANES, _LANES)
    b2 = b.reshape(C // _LANES, _LANES)

    def kernel(x_hbm, g_ref, b_ref, o_hbm, buf, gb_v, gb_s, rsem, wsem, gsem):
        def rd(a, j):
            return pltpu.make_async_copy(x_hbm.at[a, :, j], buf.at[j], rsem.at[j])

        def wr(a, j, r):
            return pltpu.make_async_copy(
                buf.at[j, :, r], o_hbm.at[a, :, j, r], wsem.at[j]
            )

        for j in range(J):
            rd(0, j).start()
        gb_v[0] = g_ref[...].astype(jnp.float32)
        gb_v[1] = b_ref[...].astype(jnp.float32)
        cp = pltpu.make_async_copy(gb_v, gb_s, gsem)
        cp.start()
        cp.wait()

        def load(j, s, r, c):
            return buf[j, s, r, :, c * CH:(c + 1) * CH].astype(jnp.float32)

        def fold(v):
            acc = v[:, 0:_LANES]
            for t in range(1, CH // _LANES):
                acc = acc + v[:, t * _LANES:(t + 1) * _LANES]
            return acc

        def compute_group(a, j):
            def body(it, carry):
                ss = [it * U + u for u in range(U)]
                mus = []
                for s in ss:
                    acc = None
                    for r in range(R):
                        for c in range(nch):
                            v = load(j, s, r, c)
                            acc = v if acc is None else acc + v
                    mus.append(jnp.sum(fold(acc), keepdims=True) * inv_n)
                affine = []
                for s, mu in zip(ss, mus):
                    acc = None
                    for r in range(R):
                        for c in range(nch):
                            d = load(j, s, r, c) - mu
                            d = d * d
                            acc = d if acc is None else acc + d
                    var = jnp.sum(fold(acc), keepdims=True) * inv_n
                    ch = lax.rem((a * S + s) * J + j, C)
                    gi = gb_s[0, ch // _LANES, ch % _LANES]
                    bi = gb_s[1, ch // _LANES, ch % _LANES]
                    sc = lax.rsqrt(var + _EPS) * gi
                    affine.append((sc, bi - mu * sc))
                for s, (sc, sh) in zip(ss, affine):
                    for r in range(R):
                        for c in range(nch):
                            y = load(j, s, r, c) * sc + sh
                            buf[j, s, r, :, c * CH:(c + 1) * CH] = y.astype(buf.dtype)
                return carry

            lax.fori_loop(0, S // U, body, 0)

        def phase(a, carry):
            def gloop(j, c2):
                @pl.when(j < M)
                def _():
                    rd(a, j).wait()

                @pl.when(j == M)
                def _():
                    for jj in range(M, J):
                        rd(a, jj).wait()
                    for jj in range(M):
                        for r in range(R):
                            wr(a, jj, r).start()

                compute_group(a, j)

                @pl.when(j >= M)
                def _():
                    for r in range(R):
                        wr(a, j, r).start()

                return c2

            lax.fori_loop(0, J, gloop, 0)
            for j in range(J):
                for r in range(R):
                    wr(a, j, r).wait()

            @pl.when(a + 1 < A)
            def _():
                for j in range(J):
                    rd(a + 1, j).start()

            return carry

        lax.fori_loop(0, A, phase, 0)

    out = pl.pallas_call(
        kernel,
        in_specs=[
            pl.BlockSpec(memory_space=pl.ANY),
            pl.BlockSpec(memory_space=pltpu.VMEM),
            pl.BlockSpec(memory_space=pltpu.VMEM),
        ],
        out_specs=pl.BlockSpec(memory_space=pl.ANY),
        out_shape=jax.ShapeDtypeStruct(xt.shape, x.dtype),
        scratch_shapes=[
            pltpu.VMEM((J, S, R, RP, H), x.dtype),
            pltpu.VMEM((2, C // _LANES, _LANES), jnp.float32),
            pltpu.SMEM((2, C // _LANES, _LANES), jnp.float32),
            pltpu.SemaphoreType.DMA((J,)),
            pltpu.SemaphoreType.DMA((J,)),
            pltpu.SemaphoreType.DMA(()),
        ],
        compiler_params=pltpu.CompilerParams(vmem_limit_bytes=100 * 1024 * 1024),
    )(xt, g2, b2)
    return jnp.transpose(out.reshape(B, C, W, H), (0, 1, 3, 2))
```

```python
import jax
import jax.numpy as jnp
from jax import lax
from jax.experimental import pallas as pl
from jax.experimental.pallas import tpu as pltpu

_EPS = 1e-5
_LANES = 128


@jax.jit
def pallas_standalone__instancenorm__prompt_kernel(
    x: jax.Array,
    g: jax.Array,
    b: jax.Array,
):
    B, C, H, W = x.shape
    N = B * C
    S = 8
    J = 8
    RP = 8
    PW = 1024
    CH = 512
    G = 11
    C0 = 2
    JH = J // 2
    R = W // RP
    HP = H // PW
    NG = N // (S * J)
    A = -(-NG // G)
    PG = S * JH
    assert NG * S * J == N and R * RP == W and HP * PW == H and H % CH == 0
    assert C % _LANES == 0 and NG - (A - 1) * G >= 2 and G <= NG
    inv_n = 1.0 / (H * W)
    nch = H // CH

    xt = jnp.transpose(x, (0, 1, 3, 2)).reshape(NG, S, J, R, RP, H)
    g2 = g.reshape(C // _LANES, _LANES)
    b2 = b.reshape(C // _LANES, _LANES)

    def kernel(x_hbm, g_hbm, b_hbm, o_hbm, buf, gb_h, gb_v, gb_s, rsem, wsem, tsem, gsem):
        def wait_bytes_of(src, dst, sem):
            pltpu.make_async_copy(src, dst, sem).wait()

        def issue_reads(a, i0, i1, low_sem=None):
            def body(i, c):
                k = i // PG
                s = (i // JH) % S
                jl = i % JH
                jh = jl + JH
                gk = a * G + k
                for r in range(R):
                    pltpu.make_async_copy(
                        x_hbm.at[gk, s, jh, r], buf.at[k, s, jh, r], rsem.at[k]
                    ).start(priority=0)
                    pltpu.make_async_copy(
                        x_hbm.at[gk, s, jl, r],
                        buf.at[k, s, jl, r],
                        rsem.at[k] if low_sem is None else low_sem,
                    ).start(priority=1)
                return c

            lax.fori_loop(i0, i1, body, 0)

        def issue_col_writes(a, k, j, r0, r1, sem):
            for r in range(r0, r1):
                for h in range(HP):
                    pltpu.make_async_copy(
                        buf.at[k, :, j, r, :, h * PW:(h + 1) * PW],
                        o_hbm.at[a * G + k, :, j, r, :, h * PW:(h + 1) * PW],
                        sem,
                    ).start()

        def total(v):
            acc = v[:, 0:_LANES]
            for t in range(1, CH // _LANES):
                acc = acc + v[:, t * _LANES:(t + 1) * _LANES]
            return jnp.sum(jnp.sum(acc, axis=1, keepdims=True), axis=0, keepdims=True)

        def normalise_col(a, k, j):
            def load(s, r, c):
                return buf[k, s, j, r, :, c * CH:(c + 1) * CH].astype(jnp.float32)

            mus = []
            for s in range(S):
                acc = None
                for r in range(R):
                    for c in range(nch):
                        v = load(s, r, c)
                        acc = v if acc is None else acc + v
                mus.append(total(acc) * inv_n)
            affine = []
            for s, mu in enumerate(mus):
                acc = None
                for r in range(R):
                    for c in range(nch):
                        d = load(s, r, c) - mu
                        d = d * d
                        acc = d if acc is None else acc + d
                var = total(acc) * inv_n
                ch = lax.rem(((a * G + k) * S + s) * J + j, C)
                row, lane = lax.div(ch, _LANES), lax.rem(ch, _LANES)
                sc = lax.rsqrt(var + _EPS) * gb_s[0, row, lane]
                affine.append((sc, gb_s[1, row, lane] - mu * sc))
            for s, (sc, sh) in enumerate(affine):
                for r in range(R):
                    for c in range(nch):
                        y = load(s, r, c) * sc + sh
                        buf[k, s, j, r, :, c * CH:(c + 1) * CH] = y.astype(buf.dtype)

        g_copy = pltpu.make_async_copy(g_hbm, gb_h.at[0], gsem.at[0])
        b_copy = pltpu.make_async_copy(b_hbm, gb_h.at[1], gsem.at[1])
        g_copy.start()
        b_copy.start()

        def phase(a, carry):
            ng = jnp.minimum(G, NG - a * G)
            last = ng - 1
            g0 = a * G
            gl = g0 + last

            issue_reads(a, 0, PG)

            @pl.when(a == 0)
            def _():
                g_copy.wait()
                b_copy.wait()
                gb_v[...] = gb_h[...].astype(jnp.float32)
                to_smem = pltpu.make_async_copy(gb_v, gb_s, gsem.at[2])
                to_smem.start()
                to_smem.wait()

            @pl.when(a > 0)
            def _():
                gp = jnp.maximum(g0 - 1, 0)
                wait_bytes_of(
                    buf.at[G - 1, :, J - 1, R - 1], o_hbm.at[gp, :, J - 1, R - 1], tsem.at[1]
                )

            issue_reads(a, PG, ng * PG - JH)
            issue_reads(a, ng * PG - JH, ng * PG, tsem.at[0])
            wait_bytes_of(x_hbm.at[g0], buf.at[0], rsem.at[0])

            def col(q, c2):
                k = q // J
                j = q % J

                @pl.when(q == C0)
                def _():
                    def wait_group(kk, c3):
                        wait_bytes_of(x_hbm.at[g0 + kk], buf.at[kk], rsem.at[kk])
                        return c3

                    lax.fori_loop(1, last, wait_group, 0)
                    wait_bytes_of(
                        x_hbm.at[gl, 0:S - 1], buf.at[last, 0:S - 1], rsem.at[last]
                    )
                    wait_bytes_of(
                        x_hbm.at[gl, S - 1, JH:J], buf.at[last, S - 1, JH:J], rsem.at[last]
                    )
                    for jj in range(C0):
                        issue_col_writes(a, 0, jj, 0, R, wsem.at[0])
                    wait_bytes_of(
                        x_hbm.at[gl, S - 1, 0:JH], buf.at[last, S - 1, 0:JH], tsem.at[0]
                    )

                normalise_col(a, k, j)

                @pl.when(q >= C0)
                def _():
                    issue_col_writes(a, k, j, 0, R - 1, wsem.at[k])

                    @pl.when(q < ng * J - 1)
                    def _():
                        issue_col_writes(a, k, j, R - 1, R, wsem.at[k])

                    @pl.when(q == ng * J - 1)
                    def _():
                        issue_col_writes(a, k, j, R - 1, R, tsem.at[1])

                return c2

            lax.fori_loop(0, ng * J, col, 0)

            def wait_writes(k, c2):
                wait_bytes_of(buf.at[k], o_hbm.at[g0 + k], wsem.at[k])
                return c2

            lax.fori_loop(0, last, wait_writes, 0)
            wait_bytes_of(buf.at[last, :, 0:J - 1], o_hbm.at[gl, :, 0:J - 1], wsem.at[last])
            wait_bytes_of(
                buf.at[last, :, J - 1, 0:R - 1], o_hbm.at[gl, :, J - 1, 0:R - 1], wsem.at[last]
            )

            @pl.when(a == A - 1)
            def _():
                wait_bytes_of(
                    buf.at[last, :, J - 1, R - 1], o_hbm.at[gl, :, J - 1, R - 1], tsem.at[1]
                )

            return carry

        lax.fori_loop(0, A, phase, 0)

    buf_bytes = G * S * J * W * H * x.dtype.itemsize
    out = pl.pallas_call(
        kernel,
        in_specs=[
            pl.BlockSpec(memory_space=pl.ANY),
            pl.BlockSpec(memory_space=pl.ANY),
            pl.BlockSpec(memory_space=pl.ANY),
        ],
        out_specs=pl.BlockSpec(memory_space=pl.ANY),
        out_shape=jax.ShapeDtypeStruct(xt.shape, x.dtype),
        scratch_shapes=[
            pltpu.VMEM((G, S, J, R, RP, H), x.dtype),
            pltpu.VMEM((2, C // _LANES, _LANES), g.dtype),
            pltpu.VMEM((2, C // _LANES, _LANES), jnp.float32),
            pltpu.SMEM((2, C // _LANES, _LANES), jnp.float32),
            pltpu.SemaphoreType.DMA((G,)),
            pltpu.SemaphoreType.DMA((G,)),
            pltpu.SemaphoreType.DMA((2,)),
            pltpu.SemaphoreType.DMA((3,)),
        ],
        compiler_params=pltpu.CompilerParams(
            vmem_limit_bytes=buf_bytes + 8 * 1024 * 1024
        ),
    )(xt, g2, b2)
    return jnp.transpose(out.reshape(B, C, W, H), (0, 1, 3, 2))
```

```python
import jax
import jax.numpy as jnp
from jax import lax
from jax.experimental import pallas as pl
from jax.experimental.pallas import tpu as pltpu

_EPS = 1e-5
_LANES = 128


@jax.jit
def pallas_standalone__instancenorm__prompt_kernel(
    x: jax.Array,
    g: jax.Array,
    b: jax.Array,
):
    B, C, H, W = x.shape
    RP = 8
    R = W // RP
    J = 8
    T = J * R
    NS = B * C // J
    RS = 8
    PR = 256
    S = 6
    PW = 1024
    G = 16
    C0 = 2
    TT = 2

    NG = NS // S
    SL = NS - NG * S
    A = -(-NG // G)
    g_end = NG - (A - 1) * G
    n_mid, n_end = G * S, g_end * S + SL
    cap = max(n_mid, n_end)
    RG = 2 * RS
    assert R * RP == W and NS * J == B * C and H % PW == 0 and H % PR == 0
    assert n_mid % RG == 0 and n_end % RG == 0 and min(n_mid, n_end) >= 2 * RG
    assert S <= RG and C0 < J and g_end >= 2 and C % _LANES == 0 and A >= 2
    inv_n = 1.0 / (H * W)

    xt = jnp.transpose(x, (0, 1, 3, 2)).reshape(NS, T, RP, H)
    g2 = g.reshape(C // _LANES, _LANES)
    b2 = b.reshape(C // _LANES, _LANES)

    def kernel(x_hbm, g_hbm, b_hbm, o_hbm, buf, gb_h, gb_v, gb_s, rsem, wsem, gsem):
        def wait_all(src, dst, sem):
            pltpu.make_async_copy(src, dst, sem).wait()

        def issue_reads(s0, i0, i1, hi_sem, lo_sem):
            def body(i, c):
                sh = RG * lax.div(i, T)
                sl = sh + RS
                t = lax.rem(i, T)
                for u in range(H // PR):
                    cols = pl.ds(u * PR, PR)
                    pltpu.make_async_copy(
                        x_hbm.at[pl.ds(s0 + sh, RS), t, :, cols],
                        buf.at[pl.ds(sh, RS), t, :, cols],
                        hi_sem,
                    ).start(priority=0)
                    pltpu.make_async_copy(
                        x_hbm.at[pl.ds(s0 + sl, RS), t, :, cols],
                        buf.at[pl.ds(sl, RS), t, :, cols],
                        lo_sem,
                    ).start(priority=1)
                return c

            lax.fori_loop(i0, i1, body, 0)

        def issue_col_writes(s0, sb, ns, j):
            for r in range(R):
                for u in range(H // PW):
                    cols = pl.ds(u * PW, PW)
                    pltpu.make_async_copy(
                        buf.at[pl.ds(sb, ns), j * R + r, :, cols],
                        o_hbm.at[pl.ds(s0 + sb, ns), j * R + r, :, cols],
                        wsem,
                    ).start()

        def total(v):
            acc = v[:, 0:_LANES]
            for u in range(1, H // _LANES):
                acc = acc + v[:, u * _LANES:(u + 1) * _LANES]
            return jnp.sum(jnp.sum(acc, axis=1, keepdims=True), axis=0, keepdims=True)

        def normalise_col(s0, sb, ns, j):
            def load(s, r):
                return buf[sb + s, j * R + r].astype(jnp.float32)

            mus = []
            for s in range(ns):
                acc = load(s, 0)
                for r in range(1, R):
                    acc = acc + load(s, r)
                mus.append(total(acc) * inv_n)
            affine = []
            for s, mu in enumerate(mus):
                acc = None
                for r in range(R):
                    d = load(s, r) - mu
                    d = d * d
                    acc = d if acc is None else acc + d
                var = total(acc) * inv_n
                ch = lax.rem((s0 + sb + s) * J + j, C)
                row, lane = lax.div(ch, _LANES), lax.rem(ch, _LANES)
                sc = lax.rsqrt(var + _EPS) * gb_s[0, row, lane]
                affine.append((sc, gb_s[1, row, lane] - mu * sc))
            for s, (sc, sh) in enumerate(affine):
                for r in range(R):
                    buf[sb + s, j * R + r] = (load(s, r) * sc + sh).astype(buf.dtype)

        g_copy = pltpu.make_async_copy(g_hbm, gb_h.at[0], gsem)
        b_copy = pltpu.make_async_copy(b_hbm, gb_h.at[1], gsem)
        to_smem = pltpu.make_async_copy(gb_v, gb_s, gsem)
        g_copy.start()
        b_copy.start()

        def phase(a, carry):
            is_end = a == A - 1
            ng = jnp.where(is_end, g_end, G)
            ni = jnp.where(is_end, n_end // RG * T, n_mid // RG * T)
            sl = jnp.where(is_end, n_end - RS, n_mid - RS)
            s0 = a * n_mid

            def with_phase_streams(f):
                pl.when(a < A - 1)(lambda: f(n_mid))
                pl.when(is_end)(lambda: f(n_end))

            issue_reads(s0, 0, T, rsem.at[0], rsem.at[0])

            @pl.when(a == 0)
            def _():
                g_copy.wait()
                b_copy.wait()
                gb_v[...] = gb_h[...].astype(jnp.float32)
                to_smem.start()

            issue_reads(s0, T, ni - T, rsem.at[1], rsem.at[1])
            issue_reads(s0, ni - T, ni - TT, rsem.at[1], rsem.at[2])
            issue_reads(s0, ni - TT, ni, rsem.at[1], rsem.at[3])

            @pl.when(a == 0)
            def _():
                to_smem.wait()

            wait_all(x_hbm.at[pl.ds(s0, RG)], buf.at[0:RG], rsem.at[0])

            def col(q, c2):
                k = lax.div(q, J)
                j = lax.rem(q, J)

                @pl.when(q == C0)
                def _():
                    with_phase_streams(
                        lambda n: wait_all(
                            x_hbm.at[pl.ds(s0 + RG, n - RS - RG)],
                            buf.at[RG:n - RS],
                            rsem.at[1],
                        )
                    )
                    wait_all(
                        x_hbm.at[pl.ds(s0 + sl, RS), 0:T - TT],
                        buf.at[pl.ds(sl, RS), 0:T - TT],
                        rsem.at[2],
                    )

                    def first(jj, c3):
                        issue_col_writes(s0, 0, S, jj)
                        return c3

                    lax.fori_loop(0, C0, first, 0)

                @pl.when(q == J)
                def _():
                    wait_all(
                        x_hbm.at[pl.ds(s0 + sl, RS), T - TT:T],
                        buf.at[pl.ds(sl, RS), T - TT:T],
                        rsem.at[3],
                    )

                normalise_col(s0, k * S, S, j)

                @pl.when(q >= C0)
                def _():
                    issue_col_writes(s0, k * S, S, j)

                return c2

            lax.fori_loop(0, ng * J, col, 0)

            if SL:

                @pl.when(is_end)
                def _():
                    def last_col(j, c2):
                        normalise_col(s0, g_end * S, SL, j)
                        issue_col_writes(s0, g_end * S, SL, j)
                        return c2

                    lax.fori_loop(0, J, last_col, 0)

            with_phase_streams(
                lambda n: wait_all(buf.at[0:n], o_hbm.at[pl.ds(s0, n)], wsem)
            )
            return carry

        lax.fori_loop(0, A, phase, 0)

    buf_bytes = cap * T * RP * H * x.dtype.itemsize
    out = pl.pallas_call(
        kernel,
        in_specs=[
            pl.BlockSpec(memory_space=pl.ANY),
            pl.BlockSpec(memory_space=pl.ANY),
            pl.BlockSpec(memory_space=pl.ANY),
        ],
        out_specs=pl.BlockSpec(memory_space=pl.ANY),
        out_shape=jax.ShapeDtypeStruct(xt.shape, x.dtype),
        scratch_shapes=[
            pltpu.VMEM((cap, T, RP, H), x.dtype),
            pltpu.VMEM((2, C // _LANES, _LANES), g.dtype),
            pltpu.VMEM((2, C // _LANES, _LANES), jnp.float32),
            pltpu.SMEM((2, C // _LANES, _LANES), jnp.float32),
            pltpu.SemaphoreType.DMA((4,)),
            pltpu.SemaphoreType.DMA(()),
            pltpu.SemaphoreType.DMA(()),
        ],
        compiler_params=pltpu.CompilerParams(
            vmem_limit_bytes=buf_bytes + 8 * 1024 * 1024
        ),
    )(xt, g2, b2)
    return jnp.transpose(out.reshape(B, C, W, H), (0, 1, 3, 2))
```

```python
import jax
import jax.numpy as jnp
from jax import lax
from jax.experimental import pallas as pl
from jax.experimental.pallas import tpu as pltpu

_EPS = 1e-5
_LANES = 128


@jax.jit
def pallas_standalone__instancenorm__prompt_kernel(
    x: jax.Array,
    g: jax.Array,
    b: jax.Array,
):
    B, C, H, W = x.shape
    RP = 8
    R = W // RP
    J = 8
    T = J * R
    NS = B * C // J
    RH = 10
    RS = 6
    PR = 256
    S = 6
    PW = 1024
    G = 16
    C0 = 2
    TT = 2

    NG = NS // S
    SL = NS - NG * S
    A = -(-NG // G)
    g_end = NG - (A - 1) * G
    n_mid, n_end = G * S, g_end * S + SL
    cap = max(n_mid, n_end)
    RG = RH + RS
    assert R * RP == W and NS * J == B * C and H % PW == 0 and H % PR == 0
    assert n_mid % RG == 0 and n_end % RG == 0 and min(n_mid, n_end) >= 2 * RG
    assert S <= RG and C0 < J and g_end >= 2 and C % _LANES == 0 and A >= 2
    inv_n = 1.0 / (H * W)

    xt = jnp.transpose(x, (0, 1, 3, 2)).reshape(NS, T, RP, H)
    g2 = g.reshape(C // _LANES, _LANES)
    b2 = b.reshape(C // _LANES, _LANES)

    def kernel(x_hbm, g_hbm, b_hbm, o_hbm, buf, gb_h, gb_v, gb_s, rsem, wsem, gsem):
        def wait_all(src, dst, sem):
            pltpu.make_async_copy(src, dst, sem).wait()

        def issue_reads(s0, i0, i1, hi_sem, lo_sem):
            def body(i, c):
                sh = RG * lax.div(i, T)
                sl = sh + RH
                t = lax.rem(i, T)
                for u in range(H // PR):
                    cols = pl.ds(u * PR, PR)
                    pltpu.make_async_copy(
                        x_hbm.at[pl.ds(s0 + sh, RH), t, :, cols],
                        buf.at[pl.ds(sh, RH), t, :, cols],
                        hi_sem,
                    ).start(priority=0)
                    pltpu.make_async_copy(
                        x_hbm.at[pl.ds(s0 + sl, RS), t, :, cols],
                        buf.at[pl.ds(sl, RS), t, :, cols],
                        lo_sem,
                    ).start(priority=1)
                return c

            lax.fori_loop(i0, i1, body, 0)

        def issue_col_writes(s0, sb, ns, j):
            for r in range(R):
                for u in range(H // PW):
                    cols = pl.ds(u * PW, PW)
                    pltpu.make_async_copy(
                        buf.at[pl.ds(sb, ns), j * R + r, :, cols],
                        o_hbm.at[pl.ds(s0 + sb, ns), j * R + r, :, cols],
                        wsem,
                    ).start()

        def total(v):
            acc = v[:, 0:_LANES]
            for u in range(1, H // _LANES):
                acc = acc + v[:, u * _LANES:(u + 1) * _LANES]
            return jnp.sum(jnp.sum(acc, axis=1, keepdims=True), axis=0, keepdims=True)

        def normalise_col(s0, sb, ns, j):
            def load(s, r):
                return buf[sb + s, j * R + r].astype(jnp.float32)

            mus = []
            for s in range(ns):
                acc = load(s, 0)
                for r in range(1, R):
                    acc = acc + load(s, r)
                mus.append(total(acc) * inv_n)
            affine = []
            for s, mu in enumerate(mus):
                acc = None
                for r in range(R):
                    d = load(s, r) - mu
                    d = d * d
                    acc = d if acc is None else acc + d
                var = total(acc) * inv_n
                ch = lax.rem((s0 + sb + s) * J + j, C)
                row, lane = lax.div(ch, _LANES), lax.rem(ch, _LANES)
                sc = lax.rsqrt(var + _EPS) * gb_s[0, row, lane]
                affine.append((sc, gb_s[1, row, lane] - mu * sc))
            for s, (sc, sh) in enumerate(affine):
                for r in range(R):
                    buf[sb + s, j * R + r] = (load(s, r) * sc + sh).astype(buf.dtype)

        g_copy = pltpu.make_async_copy(g_hbm, gb_h.at[0], gsem)
        b_copy = pltpu.make_async_copy(b_hbm, gb_h.at[1], gsem)
        to_smem = pltpu.make_async_copy(gb_v, gb_s, gsem)
        g_copy.start()
        b_copy.start()

        def phase(a, carry):
            is_end = a == A - 1
            ng = jnp.where(is_end, g_end, G)
            ni = jnp.where(is_end, n_end // RG * T, n_mid // RG * T)
            sl = jnp.where(is_end, n_end - RS, n_mid - RS)
            s0 = a * n_mid

            def with_phase_streams(f):
                pl.when(a < A - 1)(lambda: f(n_mid))
                pl.when(is_end)(lambda: f(n_end))

            issue_reads(s0, 0, T, rsem.at[0], rsem.at[0])

            @pl.when(a == 0)
            def _():
                g_copy.wait()
                b_copy.wait()
                gb_v[...] = gb_h[...].astype(jnp.float32)
                to_smem.start()

            issue_reads(s0, T, ni - T, rsem.at[1], rsem.at[1])
            issue_reads(s0, ni - T, ni - TT, rsem.at[1], rsem.at[2])
            issue_reads(s0, ni - TT, ni, rsem.at[1], rsem.at[3])

            @pl.when(a == 0)
            def _():
                to_smem.wait()

            wait_all(x_hbm.at[pl.ds(s0, RG)], buf.at[0:RG], rsem.at[0])

            def col(q, c2):
                k = lax.div(q, J)
                j = lax.rem(q, J)

                @pl.when(q == C0)
                def _():
                    with_phase_streams(
                        lambda n: wait_all(
                            x_hbm.at[pl.ds(s0 + RG, n - RS - RG)],
                            buf.at[RG:n - RS],
                            rsem.at[1],
                        )
                    )
                    wait_all(
                        x_hbm.at[pl.ds(s0 + sl, RS), 0:T - TT],
                        buf.at[pl.ds(sl, RS), 0:T - TT],
                        rsem.at[2],
                    )

                    def first(jj, c3):
                        issue_col_writes(s0, 0, S, jj)
                        return c3

                    lax.fori_loop(0, C0, first, 0)

                @pl.when(q == J)
                def _():
                    wait_all(
                        x_hbm.at[pl.ds(s0 + sl, RS), T - TT:T],
                        buf.at[pl.ds(sl, RS), T - TT:T],
                        rsem.at[3],
                    )

                normalise_col(s0, k * S, S, j)

                @pl.when(q >= C0)
                def _():
                    issue_col_writes(s0, k * S, S, j)

                return c2

            lax.fori_loop(0, ng * J, col, 0)

            if SL:

                @pl.when(is_end)
                def _():
                    def last_col(j, c2):
                        normalise_col(s0, g_end * S, SL, j)
                        issue_col_writes(s0, g_end * S, SL, j)
                        return c2

                    lax.fori_loop(0, J, last_col, 0)

            with_phase_streams(
                lambda n: wait_all(buf.at[0:n], o_hbm.at[pl.ds(s0, n)], wsem)
            )
            return carry

        lax.fori_loop(0, A, phase, 0)

    buf_bytes = cap * T * RP * H * x.dtype.itemsize
    out = pl.pallas_call(
        kernel,
        in_specs=[
            pl.BlockSpec(memory_space=pl.ANY),
            pl.BlockSpec(memory_space=pl.ANY),
            pl.BlockSpec(memory_space=pl.ANY),
        ],
        out_specs=pl.BlockSpec(memory_space=pl.ANY),
        out_shape=jax.ShapeDtypeStruct(xt.shape, x.dtype),
        scratch_shapes=[
            pltpu.VMEM((cap, T, RP, H), x.dtype),
            pltpu.VMEM((2, C // _LANES, _LANES), g.dtype),
            pltpu.VMEM((2, C // _LANES, _LANES), jnp.float32),
            pltpu.SMEM((2, C // _LANES, _LANES), jnp.float32),
            pltpu.SemaphoreType.DMA((4,)),
            pltpu.SemaphoreType.DMA(()),
            pltpu.SemaphoreType.DMA(()),
        ],
        compiler_params=pltpu.CompilerParams(
            vmem_limit_bytes=buf_bytes + 8 * 1024 * 1024
        ),
    )(xt, g2, b2)
    return jnp.transpose(out.reshape(B, C, W, H), (0, 1, 3, 2))
```

```python
import jax
import jax.numpy as jnp
from jax import lax
from jax.experimental import pallas as pl
from jax.experimental.pallas import tpu as pltpu

_EPS = 1e-5
_LANES = 128


@jax.jit
def pallas_standalone__instancenorm__prompt_kernel(
    x: jax.Array,
    g: jax.Array,
    b: jax.Array,
):
    B, C, H, W = x.shape
    RP = 8
    R = W // RP
    J = 8
    T = J * R
    NS = B * C // J
    RH = 10
    RL = 6
    PR = 256
    S = 6
    PW = 1024
    G = 16
    C0 = 2
    TT = 2

    NG = NS // S
    SL = NS - NG * S
    A = -(-NG // G)
    g_end = NG - (A - 1) * G
    n_mid, n_end = G * S, g_end * S + SL
    cap = max(n_mid, n_end)
    RG = RH + RL
    assert R * RP == W and NS * J == B * C and H % PW == 0 and H % PR == 0
    assert n_mid % RG == 0 and n_end % RG == 0 and min(n_mid, n_end) >= 3 * RG
    assert S <= RG and C0 < J and g_end >= 2 and C % _LANES == 0
    inv_n = 1.0 / (H * W)

    xt = jnp.transpose(x, (0, 1, 3, 2)).reshape(NS, T, RP, H)
    g2 = g.reshape(C // _LANES, _LANES)
    b2 = b.reshape(C // _LANES, _LANES)

    def kernel(x_hbm, g_hbm, b_hbm, o_hbm, buf, gb_h, gb_v, gb_s, rsem, wsem, gsem):
        def wait_reads(s0, sb, ns, t0, t1, sem):
            pltpu.make_async_copy(
                x_hbm.at[pl.ds(s0 + sb, ns), t0:t1], buf.at[pl.ds(sb, ns), t0:t1], sem
            ).wait()

        def wait_writes(s0, sb, ns, sem):
            pltpu.make_async_copy(
                buf.at[pl.ds(sb, ns)], o_hbm.at[pl.ds(s0 + sb, ns)], sem
            ).wait()

        def issue_reads(s0, region, t0, t1, hi_sem, lo_sem):
            sh = region * RG
            sl = sh + RH

            def body(t, c):
                for u in range(H // PR):
                    cols = pl.ds(u * PR, PR)
                    pltpu.make_async_copy(
                        x_hbm.at[pl.ds(s0 + sh, RH), t, :, cols],
                        buf.at[pl.ds(sh, RH), t, :, cols],
                        hi_sem,
                    ).start(priority=0)
                    pltpu.make_async_copy(
                        x_hbm.at[pl.ds(s0 + sl, RL), t, :, cols],
                        buf.at[pl.ds(sl, RL), t, :, cols],
                        lo_sem,
                    ).start(priority=1)
                return c

            lax.fori_loop(t0, t1, body, 0)

        def issue_col_writes(s0, sb, ns, j, sem):
            for r in range(R):
                for u in range(H // PW):
                    cols = pl.ds(u * PW, PW)
                    pltpu.make_async_copy(
                        buf.at[pl.ds(sb, ns), j * R + r, :, cols],
                        o_hbm.at[pl.ds(s0 + sb, ns), j * R + r, :, cols],
                        sem,
                    ).start()

        def mean(v):
            v = jnp.sum(jnp.sum(v, axis=0), axis=1, keepdims=True)
            return jnp.sum(v, axis=0, keepdims=True) * inv_n

        def normalise_col(s0, sb, ns, j):
            rows = pl.ds(j * R, R)

            def load(s):
                return buf[sb + s, rows].astype(jnp.float32)

            mus = [mean(load(s)) for s in range(ns)]
            affine = []
            for s, mu in enumerate(mus):
                d = load(s) - mu
                var = mean(d * d)
                ch = lax.rem((s0 + sb + s) * J + j, C)
                row, lane = lax.div(ch, _LANES), lax.rem(ch, _LANES)
                sc = lax.rsqrt(var + _EPS) * gb_s[0, row, lane]
                affine.append((sc, gb_s[1, row, lane] - mu * sc))
            for s, (sc, sh) in enumerate(affine):
                buf[sb + s, rows] = (load(s) * sc + sh).astype(buf.dtype)

        g_copy = pltpu.make_async_copy(g_hbm, gb_h.at[0], gsem)
        b_copy = pltpu.make_async_copy(b_hbm, gb_h.at[1], gsem)
        to_smem = pltpu.make_async_copy(gb_v, gb_s, gsem)
        g_copy.start()
        b_copy.start()

        def phase(a, carry):
            is_end = a == A - 1
            ng = jnp.where(is_end, g_end, G)
            last = jnp.where(is_end, n_end // RG - 1, n_mid // RG - 1)
            s0 = a * n_mid

            def read_region(i, c2):
                sem = rsem.at[lax.rem(i, 2)]

                @pl.when(i >= 2)
                def _():
                    wait_reads(s0, (i - 2) * RG, RG, 0, T, sem)

                @pl.when(jnp.logical_and(a == 0, i == 1))
                def _():
                    g_copy.wait()
                    b_copy.wait()
                    gb_v[...] = gb_h[...].astype(jnp.float32)
                    to_smem.start()

                lo_sem = rsem.at[jnp.where(i == last, 2, lax.rem(i, 2))]
                issue_reads(s0, i, 0, jnp.where(i == last, T - TT, T), sem, lo_sem)
                return c2

            lax.fori_loop(0, last + 1, read_region, 0)
            issue_reads(s0, last, T - TT, T, rsem.at[lax.rem(last, 2)], rsem.at[3])

            @pl.when(a == 0)
            def _():
                to_smem.wait()

            def col(q, c2):
                k = lax.div(q, J)
                j = lax.rem(q, J)
                sem = wsem.at[lax.rem(k, 2)]

                @pl.when(q == C0)
                def _():
                    wait_reads(s0, (last - 1) * RG, RG, 0, T, rsem.at[lax.rem(last - 1, 2)])
                    wait_reads(s0, last * RG, RH, 0, T, rsem.at[lax.rem(last, 2)])
                    wait_reads(s0, last * RG + RH, RL, 0, T - TT, rsem.at[2])

                    def first(jj, c3):
                        issue_col_writes(s0, 0, S, jj, wsem.at[0])
                        return c3

                    lax.fori_loop(0, C0, first, 0)

                @pl.when(q == J)
                def _():
                    wait_reads(s0, last * RG + RH, RL, T - TT, T, rsem.at[3])

                @pl.when(jnp.logical_and(j == 0, k >= 2))
                def _():
                    wait_writes(s0, (k - 2) * S, S, sem)

                normalise_col(s0, k * S, S, j)

                @pl.when(q >= C0)
                def _():
                    issue_col_writes(s0, k * S, S, j, sem)

                return c2

            lax.fori_loop(0, ng * J, col, 0)
            wait_writes(s0, (ng - 2) * S, S, wsem.at[lax.rem(ng, 2)])

            if SL:

                @pl.when(is_end)
                def _():
                    def last_col(j, c2):
                        normalise_col(s0, g_end * S, SL, j)
                        issue_col_writes(s0, g_end * S, SL, j, wsem.at[g_end % 2])
                        return c2

                    lax.fori_loop(0, J, last_col, 0)

            wait_writes(s0, (ng - 1) * S, S, wsem.at[lax.rem(ng - 1, 2)])

            if SL:

                @pl.when(is_end)
                def _():
                    wait_writes(s0, g_end * S, SL, wsem.at[g_end % 2])

            return carry

        lax.fori_loop(0, A, phase, 0)

    buf_bytes = cap * T * RP * H * x.dtype.itemsize
    out = pl.pallas_call(
        kernel,
        in_specs=[
            pl.BlockSpec(memory_space=pl.ANY),
            pl.BlockSpec(memory_space=pl.ANY),
            pl.BlockSpec(memory_space=pl.ANY),
        ],
        out_specs=pl.BlockSpec(memory_space=pl.ANY),
        out_shape=jax.ShapeDtypeStruct(xt.shape, x.dtype),
        scratch_shapes=[
            pltpu.VMEM((cap, T, RP, H), x.dtype),
            pltpu.VMEM((2, C // _LANES, _LANES), g.dtype),
            pltpu.VMEM((2, C // _LANES, _LANES), jnp.float32),
            pltpu.SMEM((2, C // _LANES, _LANES), jnp.float32),
            pltpu.SemaphoreType.DMA((4,)),
            pltpu.SemaphoreType.DMA((2,)),
            pltpu.SemaphoreType.DMA(()),
        ],
        compiler_params=pltpu.CompilerParams(
            vmem_limit_bytes=buf_bytes + 8 * 1024 * 1024
        ),
    )(xt, g2, b2)
    return jnp.transpose(out.reshape(B, C, W, H), (0, 1, 3, 2))
```

```python
import jax
import jax.numpy as jnp
from jax import lax
from jax.experimental import pallas as pl
from jax.experimental.pallas import tpu as pltpu

_EPS = 1e-5
_LANES = 128


@jax.jit
def pallas_standalone__instancenorm__prompt_kernel(
    x: jax.Array,
    g: jax.Array,
    b: jax.Array,
):
    B, C, H, W = x.shape
    RP = 8
    R = W // RP
    J = 8
    T = J * R
    NS = B * C // J
    RH = 10
    RL = 6
    PR = 256
    S = 6
    PW = 1024
    G = 16
    C0 = 2
    TT = 2

    NG = NS // S
    SL = NS - NG * S
    A = -(-NG // G)
    g_end = NG - (A - 1) * G
    n_mid, n_end = G * S, g_end * S + SL
    cap = max(n_mid, n_end)
    RG = RH + RL
    assert R * RP == W and NS * J == B * C and H % PW == 0 and H % PR == 0
    assert n_mid % RG == 0 and n_end % RG == 0 and min(n_mid, n_end) >= 3 * RG
    assert S <= RG and C0 < J and g_end >= 2 and C % _LANES == 0
    inv_n = 1.0 / (H * W)

    xt = jnp.transpose(x, (0, 1, 3, 2)).reshape(NS, T, RP, H)
    g2 = g.reshape(C // _LANES, _LANES)
    b2 = b.reshape(C // _LANES, _LANES)

    def kernel(x_hbm, g_hbm, b_hbm, o_hbm, buf, gb_h, gb_v, gb_s, rsem, wsem, gsem):
        def wait_reads(s0, sb, ns, t0, t1, sem):
            pltpu.make_async_copy(
                x_hbm.at[pl.ds(s0 + sb, ns), t0:t1], buf.at[pl.ds(sb, ns), t0:t1], sem
            ).wait()

        def wait_writes(s0, sb, ns, sem):
            pltpu.make_async_copy(
                buf.at[pl.ds(sb, ns)], o_hbm.at[pl.ds(s0 + sb, ns)], sem
            ).wait()

        def issue_reads(s0, region, t0, t1, hi_sem, lo_sem):
            sh = region * RG
            sl = sh + RH

            def body(t, c):
                for u in range(H // PR):
                    cols = pl.ds(u * PR, PR)
                    pltpu.make_async_copy(
                        x_hbm.at[pl.ds(s0 + sh, RH), t, :, cols],
                        buf.at[pl.ds(sh, RH), t, :, cols],
                        hi_sem,
                    ).start(priority=0)
                    pltpu.make_async_copy(
                        x_hbm.at[pl.ds(s0 + sl, RL), t, :, cols],
                        buf.at[pl.ds(sl, RL), t, :, cols],
                        lo_sem,
                    ).start(priority=1)
                return c

            lax.fori_loop(t0, t1, body, 0)

        def issue_col_writes(s0, sb, ns, j, sem):
            for r in range(R):
                for u in range(H // PW):
                    cols = pl.ds(u * PW, PW)
                    pltpu.make_async_copy(
                        buf.at[pl.ds(sb, ns), j * R + r, :, cols],
                        o_hbm.at[pl.ds(s0 + sb, ns), j * R + r, :, cols],
                        sem,
                    ).start()

        def mean(v):
            v = jnp.sum(jnp.sum(v, axis=0), axis=1, keepdims=True)
            return jnp.sum(v, axis=0, keepdims=True) * inv_n

        def normalise_col(s0, sb, ns, j):
            rows = pl.ds(j * R, R)
            xs = [buf[sb + s, rows].astype(jnp.float32) for s in range(ns)]
            ds = [v - mean(v) for v in xs]
            rstds = [lax.rsqrt(mean(d * d) + _EPS) for d in ds]
            for s in range(ns):
                ch = lax.rem((s0 + sb + s) * J + j, C)
                row, lane = lax.div(ch, _LANES), lax.rem(ch, _LANES)
                y = ds[s] * (rstds[s] * gb_s[0, row, lane]) + gb_s[1, row, lane]
                buf[sb + s, rows] = y.astype(buf.dtype)

        g_copy = pltpu.make_async_copy(g_hbm, gb_h.at[0], gsem)
        b_copy = pltpu.make_async_copy(b_hbm, gb_h.at[1], gsem)
        to_smem = pltpu.make_async_copy(gb_v, gb_s, gsem)
        g_copy.start()
        b_copy.start()

        def phase(a, carry):
            is_end = a == A - 1
            ng = jnp.where(is_end, g_end, G)
            last = jnp.where(is_end, n_end // RG - 1, n_mid // RG - 1)
            s0 = a * n_mid

            def read_region(i, c2):
                sem = rsem.at[lax.rem(i, 2)]

                @pl.when(i >= 2)
                def _():
                    wait_reads(s0, (i - 2) * RG, RG, 0, T, sem)

                @pl.when(jnp.logical_and(a == 0, i == 1))
                def _():
                    g_copy.wait()
                    b_copy.wait()
                    gb_v[...] = gb_h[...].astype(jnp.float32)
                    to_smem.start()

                lo_sem = rsem.at[jnp.where(i == last, 2, lax.rem(i, 2))]
                issue_reads(s0, i, 0, jnp.where(i == last, T - TT, T), sem, lo_sem)
                return c2

            lax.fori_loop(0, last + 1, read_region, 0)
            issue_reads(s0, last, T - TT, T, rsem.at[lax.rem(last, 2)], rsem.at[3])

            @pl.when(a == 0)
            def _():
                to_smem.wait()

            def col(q, c2):
                k = lax.div(q, J)
                j = lax.rem(q, J)
                sem = wsem.at[lax.rem(k, 2)]

                @pl.when(q == C0)
                def _():
                    wait_reads(s0, (last - 1) * RG, RG, 0, T, rsem.at[lax.rem(last - 1, 2)])
                    wait_reads(s0, last * RG, RH, 0, T, rsem.at[lax.rem(last, 2)])
                    wait_reads(s0, last * RG + RH, RL, 0, T - TT, rsem.at[2])

                    def first(jj, c3):
                        issue_col_writes(s0, 0, S, jj, wsem.at[0])
                        return c3

                    lax.fori_loop(0, C0, first, 0)

                @pl.when(q == J)
                def _():
                    wait_reads(s0, last * RG + RH, RL, T - TT, T, rsem.at[3])

                @pl.when(jnp.logical_and(j == 0, k >= 2))
                def _():
                    wait_writes(s0, (k - 2) * S, S, sem)

                normalise_col(s0, k * S, S, j)

                @pl.when(q >= C0)
                def _():
                    issue_col_writes(s0, k * S, S, j, sem)

                return c2

            lax.fori_loop(0, ng * J, col, 0)
            wait_writes(s0, (ng - 2) * S, S, wsem.at[lax.rem(ng, 2)])

            if SL:

                @pl.when(is_end)
                def _():
                    def last_col(j, c2):
                        normalise_col(s0, g_end * S, SL, j)
                        issue_col_writes(s0, g_end * S, SL, j, wsem.at[g_end % 2])
                        return c2

                    lax.fori_loop(0, J, last_col, 0)

            wait_writes(s0, (ng - 1) * S, S, wsem.at[lax.rem(ng - 1, 2)])

            if SL:

                @pl.when(is_end)
                def _():
                    wait_writes(s0, g_end * S, SL, wsem.at[g_end % 2])

            return carry

        lax.fori_loop(0, A, phase, 0)

    buf_bytes = cap * T * RP * H * x.dtype.itemsize
    out = pl.pallas_call(
        kernel,
        in_specs=[
            pl.BlockSpec(memory_space=pl.ANY),
            pl.BlockSpec(memory_space=pl.ANY),
            pl.BlockSpec(memory_space=pl.ANY),
        ],
        out_specs=pl.BlockSpec(memory_space=pl.ANY),
        out_shape=jax.ShapeDtypeStruct(xt.shape, x.dtype),
        scratch_shapes=[
            pltpu.VMEM((cap, T, RP, H), x.dtype),
            pltpu.VMEM((2, C // _LANES, _LANES), g.dtype),
            pltpu.VMEM((2, C // _LANES, _LANES), jnp.float32),
            pltpu.SMEM((2, C // _LANES, _LANES), jnp.float32),
            pltpu.SemaphoreType.DMA((4,)),
            pltpu.SemaphoreType.DMA((2,)),
            pltpu.SemaphoreType.DMA(()),
        ],
        compiler_params=pltpu.CompilerParams(
            vmem_limit_bytes=buf_bytes + 8 * 1024 * 1024
        ),
    )(xt, g2, b2)
    return jnp.transpose(out.reshape(B, C, W, H), (0, 1, 3, 2))
```
